```python
import os as _os
_os.environ.setdefault("JAX_PLATFORMS", "cpu")
import jax
import jax.numpy as jnp

def _softmax(x, axis=-1):
    return jax.nn.softmax(x, axis=axis)
def _gelu(x):
    return jax.nn.gelu(x, approximate=True)
def _silu(x):
    return jax.nn.silu(x)
def _sigmoid(x):
    return jax.nn.sigmoid(x)
def _layernorm(x, axis=-1, eps=1e-5):
    m = jnp.mean(x, axis=axis, keepdims=True)
    v = jnp.var(x, axis=axis, keepdims=True)
    return (x - m) / jnp.sqrt(v + eps)
def _scatter_add(tgt, idx, src, axis=0):
    return tgt.at[idx].add(src)
def _segment_sum(src, seg, n):
    return jax.ops.segment_sum(src, seg, n)
class _Rng:
    def __init__(self, key):
        self._k = key
    def _next(self):
        self._k, sub = jax.random.split(self._k)
        return sub
    def normal(self, shape):
        return jax.random.normal(self._next(), shape, dtype=jnp.bfloat16)
    def randint(self, lo, hi, shape):
        return jax.random.randint(self._next(), shape, lo, hi, dtype=jnp.int32)
    def uniform(self, shape, lo=0.0, hi=1.0):
        return jax.random.uniform(self._next(), shape, jnp.bfloat16, lo, hi)
    def permutation(self, n):
        return jax.random.permutation(self._next(), n)


kernel_name = 'parallel_sum__ssm_conv_h3__dense_activation_silu__prompt'

def setup_inputs():
    _rng = _Rng(jax.random.key(int.from_bytes(__import__("os").urandom(4), "little")))
    _w = (lambda a: (lambda t: t.astype(jnp.bfloat16) if jnp.issubdtype(t.dtype, jnp.floating) else t)(jnp.asarray(a)))
    def _A_setup():
        B, S, D = 1, 2048, 448
        ks = 4
        return {
            "q": _w((lambda *s: _rng.normal(s) * 0.05)(B, S, D)),
            "k": _w((lambda *s: _rng.normal(s) * 0.2)(B, S, D)),
            "v": _w((lambda *s: _rng.normal(s) * 0.2)(B, S, D)),
            "shift_k": _w((lambda *s: _rng.normal(s) * 0.2)(D, ks) * 0.5),
            "ssm_k": _w((lambda *s: _rng.normal(s) * 0.2)(D, S) * (1.0 / S ** 0.5)),
            "ssm_D": _w((lambda *s: _rng.normal(s) * 0.2)(D)),
        }
    _A_in = _A_setup()

    def _B_setup():
        B, S, D, F = 1, 2048, 448, 1792
        return {
            "x": _w((lambda *s: _rng.normal(s) * 0.05)(B, S, D)),
            "w1": _w((lambda *s: _rng.normal(s) * 0.05)(D, F) * (D ** -0.5)),
            "w2": _w((lambda *s: _rng.normal(s) * 0.05)(F, D) * (F ** -0.5)),
        }
    _B_in = _B_setup()

    return {
        "A_q": _A_in["q"],
        "A_k": _A_in["k"],
        "A_v": _A_in["v"],
        "A_shift_k": _A_in["shift_k"],
        "A_ssm_k": _A_in["ssm_k"],
        "A_ssm_D": _A_in["ssm_D"],
        "B_x": _B_in["x"],
        "B_w1": _B_in["w1"],
        "B_w2": _B_in["w2"],
    }

def reference(A_q, A_k, A_v, A_shift_k, A_ssm_k, A_ssm_D, B_x, B_w1, B_w2):
    def _A_ref(q, k, v, shift_k, ssm_k, ssm_D):
        B, S, D = q.shape
        ks = shift_k.shape[-1]
        k_pad = jnp.pad(k, ((0, 0), (ks - 1, 0), (0, 0)))
        k_shift = jnp.zeros_like(k)
        for t in range(ks):
            k_shift = k_shift + k_pad[:, t:t + S, :] * shift_k[:, ks - 1 - t][None, None, :]
        kv = k_shift * v
        L = 2 * S
        kv_pad = jnp.pad(kv, ((0, 0), (0, S), (0, 0)))
        kf_pad = jnp.pad(ssm_k, ((0, 0), (0, S)))
        kv_f = (lambda x, axes=(-2,-1): jnp.fft.rfft2(x.astype(jnp.float32), axes=axes))(kv_pad[:, None, :, :], axes=(1, 2))
        kf_f = (lambda x, axes=(-2,-1): jnp.fft.rfft2(x.astype(jnp.float32), axes=axes))(kf_pad[:, None, :], axes=(1, 2))
        kf_f = (lambda x, *d: x.transpose(*d))(kf_f, 1, 2, 0)
        y_f = kv_f * kf_f[None, :, :, :]
        y = (lambda x, s, axes=(-2,-1): jnp.fft.irfft2(x, s=s, axes=axes).astype(jnp.bfloat16))(y_f, (1, L), axes=(1, 2))[:, 0, :S, :]
        y = y + kv * ssm_D[None, None, :]
        return q * y

    def _B_ref(x, w1, w2):
        h = jnp.einsum("bsd,df->bsf", x, w1)
        h = _silu(h)
        out = jnp.einsum("bsf,fd->bsd", h, w2)
        return out

    x = A_q
    xn = _layernorm(x, axis=-1)
    return x + _A_ref(xn, A_k, A_v, A_shift_k, A_ssm_k, A_ssm_D) + _B_ref(xn, B_w1, B_w2)
```

```python
import functools

import numpy as np
import jax
import jax.numpy as jnp
from jax import lax
import jax.experimental.pallas as pl
import jax.experimental.pallas.tpu as pltpu

C = 128
N2 = 2 * C
STRIP = 16
EPS = 1e-5


def _dft_constants():
    f = np.arange(C, dtype=np.float64)[:, None] + 0.5
    t = np.arange(C, dtype=np.float64)[None, :]
    ang = 2.0 * np.pi * f * t / N2
    fwd = np.concatenate([np.cos(ang), -np.sin(ang)], axis=0)
    n = np.arange(C, dtype=np.float64)[:, None] + C
    fb = np.arange(C, dtype=np.float64)[None, :] + 0.5
    angi = 2.0 * np.pi * n * fb / N2
    inv = np.concatenate([np.cos(angi), -np.sin(angi)], axis=1) * (2.0 / N2)
    sgn = np.where(np.arange(C) % 2 == 0, 1.0, -1.0)[:, None]
    return fwd, inv, sgn


def _kernel(x_ref, k_ref, v_ref, sk_ref, h_ref, d_ref, w1_ref, w2_ref,
            fwd_ref, inv_ref, sgn_ref,
            o_ref,
            hf_ref, uf_ref, uprev_ref, kprev_ref, y_ref):
    i = pl.program_id(0)
    D = x_ref.shape[-1]
    f32 = jnp.float32
    bf16 = jnp.bfloat16

    @pl.when(i == 0)
    def _():
        uprev_ref[...] = jnp.zeros(uprev_ref.shape, f32)
        kprev_ref[...] = jnp.zeros(kprev_ref.shape, f32)

    x = x_ref[...].astype(f32)
    m = jnp.mean(x, axis=-1, keepdims=True)
    xc = x - m
    var = jnp.mean(xc * xc, axis=-1, keepdims=True)
    xn = xc * lax.rsqrt(var + EPS)
    xn_b = xn.astype(bf16)

    kf = k_ref[...].astype(f32)
    ext = jnp.concatenate([kprev_ref[...], kf], axis=0)
    sk = sk_ref[...].astype(f32)
    ksh = kf * sk[0:1, :]
    for t in range(1, 4):
        ksh = ksh + ext[8 - t:8 - t + C, :] * sk[t:t + 1, :]
    kprev_ref[...] = kf[C - 8:, :]
    kv = ksh * v_ref[...].astype(f32)
    kv_b = kv.astype(bf16)

    fwd = fwd_ref[...]
    u = jnp.dot(fwd, kv_b, preferred_element_type=f32)
    hh = lax.dot_general(fwd, h_ref[...], (((1,), (1,)), ((), ())),
                         preferred_element_type=f32)
    hf_ref[i] = hh
    sgn = sgn_ref[...]
    ur, ui = u[:C], u[C:]
    up = uprev_ref[...]
    uf_ref[i, :C, :] = up[:C] + sgn * ui
    uf_ref[i, C:, :] = up[C:] - sgn * ur
    uprev_ref[...] = u

    def strip_body(r, carry):
        r0 = pl.multiple_of(r * STRIP, STRIP)
        rr = pl.ds(r0, STRIP)
        ri = pl.ds(r0 + C, STRIP)

        def body(kk, acc):
            ar, ai = acc
            hr = hf_ref[kk, rr, :]
            hi = hf_ref[kk, ri, :]
            wr = uf_ref[i - kk, rr, :]
            wi = uf_ref[i - kk, ri, :]
            return (ar + (hr * wr - hi * wi), ai + (hr * wi + hi * wr))

        z = jnp.zeros((STRIP, D), f32)
        ar, ai = lax.fori_loop(0, i + 1, body, (z, z))
        y_ref[rr, :] = ar.astype(bf16)
        y_ref[ri, :] = ai.astype(bf16)
        return carry

    lax.fori_loop(0, C // STRIP, strip_body, 0)
    y = jnp.dot(inv_ref[...], y_ref[...], preferred_element_type=f32)
    y = y + kv * d_ref[...].astype(f32)
    a_out = xn * y

    h1 = jnp.dot(xn_b, w1_ref[...], preferred_element_type=f32)
    h1 = h1 * jax.nn.sigmoid(h1)
    b_out = jnp.dot(h1.astype(bf16), w2_ref[...], preferred_element_type=f32)

    o_ref[...] = (x + a_out + b_out).astype(o_ref.dtype)


@jax.jit
def pallas_parallel_sum__ssm_conv_h3__dense_activation_silu__prompt_kernel(
    A_q: jax.Array,
    A_k: jax.Array,
    A_v: jax.Array,
    A_shift_k: jax.Array,
    A_ssm_k: jax.Array,
    A_ssm_D: jax.Array,
    B_x: jax.Array,
    B_w1: jax.Array,
    B_w2: jax.Array,
):
    B, S, D = A_q.shape
    assert B == 1 and S % C == 0
    F = B_w1.shape[1]
    nb = S // C
    bf16 = jnp.bfloat16

    x2 = A_q.reshape(S, D)
    k2 = A_k.reshape(S, D)
    v2 = A_v.reshape(S, D)
    sk = jnp.pad(A_shift_k.T, ((0, 4), (0, 0)))
    d2 = A_ssm_D.reshape(1, D)

    fwd, inv, sgn = _dft_constants()
    fwd = jnp.asarray(fwd, dtype=bf16)
    inv = jnp.asarray(inv, dtype=bf16)
    sgn = jnp.asarray(sgn, dtype=jnp.float32)

    row = lambda i: (i, 0)
    const = lambda i: (0, 0)
    out = pl.pallas_call(
        _kernel,
        grid=(nb,),
        in_specs=[
            pl.BlockSpec((C, D), row),
            pl.BlockSpec((C, D), row),
            pl.BlockSpec((C, D), row),
            pl.BlockSpec((8, D), const),
            pl.BlockSpec((D, C), lambda i: (0, i)),
            pl.BlockSpec((1, D), const),
            pl.BlockSpec((D, F), const),
            pl.BlockSpec((F, D), const),
            pl.BlockSpec((N2, C), const),
            pl.BlockSpec((C, N2), const),
            pl.BlockSpec((C, 1), const),
        ],
        out_specs=pl.BlockSpec((C, D), row),
        out_shape=jax.ShapeDtypeStruct((S, D), A_q.dtype),
        scratch_shapes=[
            pltpu.VMEM((nb, N2, D), jnp.float32),
            pltpu.VMEM((nb, N2, D), jnp.float32),
            pltpu.VMEM((N2, D), jnp.float32),
            pltpu.VMEM((8, D), jnp.float32),
            pltpu.VMEM((N2, D), bf16),
        ],
        compiler_params=pltpu.CompilerParams(
            dimension_semantics=("arbitrary",),
            vmem_limit_bytes=100 * 1024 * 1024,
        ),
    )(x2, k2, v2, sk, A_ssm_k, d2, B_w1, B_w2, fwd, inv, sgn)
    return out.reshape(B, S, D)
```

```python
import numpy as np
import jax
import jax.numpy as jnp
from jax import lax
import jax.experimental.pallas as pl
import jax.experimental.pallas.tpu as pltpu

C = 128
N2 = 2 * C
SUB = 2
W = SUB * C
STRIP = 32
EPS = 1e-5


def _dft_constants():
    t = np.arange(C, dtype=np.float64)[:, None]
    f = np.arange(C, dtype=np.float64)[None, :] + 0.5
    ang = 2.0 * np.pi * t * f / N2
    fwd = np.concatenate([np.cos(ang), -np.sin(ang)], axis=1)
    fb = np.arange(C, dtype=np.float64)[:, None] + 0.5
    n = np.arange(C, dtype=np.float64)[None, :] + C
    angi = 2.0 * np.pi * fb * n / N2
    inv = np.concatenate([np.cos(angi), -np.sin(angi)], axis=0) * (2.0 / N2)
    sgn = np.where(np.arange(C) % 2 == 0, 1.0, -1.0)[None, :]
    return fwd, inv, sgn


def _kernel(x_ref, k_ref, v_ref, sk_ref, h_ref, d_ref, w1_ref, w2t_ref,
            fwd_ref, inv_ref, sgn_ref,
            o_ref,
            hf_ref, uf_ref, uprev_ref, kprev_ref, yacc_ref, w1t_ref):
    step = pl.program_id(0)
    D = x_ref.shape[0]
    f32 = jnp.float32
    bf16 = jnp.bfloat16

    @pl.when(step == 0)
    def _():
        uprev_ref[...] = jnp.zeros(uprev_ref.shape, f32)
        kprev_ref[...] = jnp.zeros(kprev_ref.shape, f32)
        w1t_ref[...] = w1_ref[...].T

    x = x_ref[...].astype(f32)
    m = jnp.mean(x, axis=0, keepdims=True)
    xc = x - m
    var = jnp.mean(xc * xc, axis=0, keepdims=True)
    xn = xc * lax.rsqrt(var + EPS)
    xn_b = xn.astype(bf16)

    sk = sk_ref[...].astype(f32)
    dd = d_ref[...].astype(f32)
    lane = lax.broadcasted_iota(jnp.int32, (D, C), 1)
    fwd = fwd_ref[...]
    sgn = sgn_ref[...]

    ys = []
    bs = []
    for sub in range(SUB):
        i = step * SUB + sub
        cols = slice(sub * C, (sub + 1) * C)
        h1 = jnp.dot(w1t_ref[...], xn_b[:, cols], preferred_element_type=f32)
        h1 = h1 * (0.5 + 0.5 * jnp.tanh(0.5 * h1))
        bs.append(jnp.dot(w2t_ref[...], h1.astype(bf16), preferred_element_type=f32))
        kf = k_ref[:, cols].astype(f32)
        ksh = kf * sk[:, 0:1]
        for t in range(1, 4):
            rolled = pltpu.roll(kf, t, 1)
            sh = jnp.where(lane < t, kprev_ref[t - 1], rolled)
            kprev_ref[t - 1] = rolled
            ksh = ksh + sh * sk[:, t:t + 1]
        kv = ksh * v_ref[:, cols].astype(f32)
        kv_b = kv.astype(bf16)

        u = jnp.dot(kv_b, fwd, preferred_element_type=f32)
        hf_ref[i] = jnp.dot(h_ref[:, cols], fwd, preferred_element_type=f32)
        up = uprev_ref[...]
        uf_ref[i, :, :C] = up[:, :C] + sgn * u[:, C:]
        uf_ref[i, :, C:] = up[:, C:] - sgn * u[:, :C]
        uprev_ref[...] = u

        def mac(terms, init):
            for r in range(D // STRIP):
                rows = slice(r * STRIP, (r + 1) * STRIP)
                ar = None if init else yacc_ref[rows, :C]
                ai = None if init else yacc_ref[rows, C:]
                for kk in terms:
                    hr = hf_ref[kk, rows, :C]
                    hi = hf_ref[kk, rows, C:]
                    wr = uf_ref[i - kk, rows, :C]
                    wi = uf_ref[i - kk, rows, C:]
                    pr = hr * wr - hi * wi
                    pi = hr * wi + hi * wr
                    ar = pr if ar is None else ar + pr
                    ai = pi if ai is None else ai + pi
                yacc_ref[rows, :C] = ar
                yacc_ref[rows, C:] = ai

        nfirst = 1 + sub
        mac(tuple(range(nfirst)), True)

        def pair_body(j, carry):
            k0 = nfirst + 2 * j
            mac((k0, k0 + 1), False)
            return carry

        lax.fori_loop(0, step, pair_body, 0)

        y = jnp.dot(yacc_ref[...].astype(bf16), inv_ref[...], preferred_element_type=f32)
        ys.append(y + kv * dd)

    a_out = xn * jnp.concatenate(ys, axis=1)

    b_out = jnp.concatenate(bs, axis=1)
    o_ref[...] = (x + a_out + b_out).astype(o_ref.dtype)


@jax.jit
def pallas_parallel_sum__ssm_conv_h3__dense_activation_silu__prompt_kernel(
    A_q: jax.Array,
    A_k: jax.Array,
    A_v: jax.Array,
    A_shift_k: jax.Array,
    A_ssm_k: jax.Array,
    A_ssm_D: jax.Array,
    B_x: jax.Array,
    B_w1: jax.Array,
    B_w2: jax.Array,
):
    B, S, D = A_q.shape
    assert B == 1 and S % W == 0
    F = B_w1.shape[1]
    nb = S // C
    bf16 = jnp.bfloat16

    xt = A_q.reshape(S, D).T
    kt = A_k.reshape(S, D).T
    vt = A_v.reshape(S, D).T
    d2 = A_ssm_D.reshape(D, 1)
    w2t = B_w2.T

    fwd, inv, sgn = _dft_constants()
    fwd = jnp.asarray(fwd, dtype=bf16)
    inv = jnp.asarray(inv, dtype=bf16)
    sgn = jnp.asarray(sgn, dtype=jnp.float32)

    col = lambda i: (0, i)
    const = lambda i: (0, 0)
    out = pl.pallas_call(
        _kernel,
        grid=(S // W,),
        in_specs=[
            pl.BlockSpec((D, W), col),
            pl.BlockSpec((D, W), col),
            pl.BlockSpec((D, W), col),
            pl.BlockSpec((D, 4), const),
            pl.BlockSpec((D, W), col),
            pl.BlockSpec((D, 1), const),
            pl.BlockSpec((D, F), const),
            pl.BlockSpec((D, F), const),
            pl.BlockSpec((C, N2), const),
            pl.BlockSpec((N2, C), const),
            pl.BlockSpec((1, C), const),
        ],
        out_specs=pl.BlockSpec((D, W), col),
        out_shape=jax.ShapeDtypeStruct((D, S), A_q.dtype),
        scratch_shapes=[
            pltpu.VMEM((nb, D, N2), jnp.float32),
            pltpu.VMEM((nb, D, N2), jnp.float32),
            pltpu.VMEM((D, N2), jnp.float32),
            pltpu.VMEM((3, D, C), jnp.float32),
            pltpu.VMEM((D, N2), jnp.float32),
            pltpu.VMEM((F, D), bf16),
        ],
        compiler_params=pltpu.CompilerParams(
            dimension_semantics=("arbitrary",),
            vmem_limit_bytes=100 * 1024 * 1024,
        ),
    )(xt, kt, vt, A_shift_k, A_ssm_k, d2, B_w1, w2t, fwd, inv, sgn)
    return out.T.reshape(B, S, D)
```

```python
import numpy as np
import jax
import jax.numpy as jnp
from jax import lax
import jax.experimental.pallas as pl
import jax.experimental.pallas.tpu as pltpu

C = 128
N2 = 2 * C
SUB = 2
W = SUB * C
STRIP = 16
EPS = 1e-5
ES = 64


def _dft_constants():
    t = np.arange(C, dtype=np.float64)[:, None]
    f = np.arange(C, dtype=np.float64)[None, :] + 0.5
    ang = 2.0 * np.pi * t * f / N2
    fwd = np.concatenate([np.cos(ang), -np.sin(ang)], axis=1)
    fb = np.arange(C, dtype=np.float64)[:, None] + 0.5
    n = np.arange(C, dtype=np.float64)[None, :] + C
    angi = 2.0 * np.pi * fb * n / N2
    inv = np.concatenate([np.cos(angi), -np.sin(angi)], axis=0) * (2.0 / N2)
    sgn = np.where(np.arange(C) % 2 == 0, 1.0, -1.0)[None, :]
    return fwd, inv, sgn


def _kernel(x_ref, k_ref, v_ref, sk_ref, h_ref, d_ref, w1_ref, w2t_ref,
            fwd_ref, inv_ref, sgn_ref,
            o_ref,
            hf_ref, uf_ref, uprev_ref, kprev_ref, yacc_ref, w1t_ref, xnb_ref, kvb_ref, bout_ref):
    step = pl.program_id(0)
    D = x_ref.shape[0]
    f32 = jnp.float32
    bf16 = jnp.bfloat16

    @pl.when(step == 0)
    def _():
        uprev_ref[...] = jnp.zeros(uprev_ref.shape, f32)
        kprev_ref[...] = jnp.zeros(kprev_ref.shape, f32)
        w1t_ref[...] = w1_ref[...].T

    nst = D // ES

    def strip(r):
        return slice(r * ES, (r + 1) * ES)

    ssum = None
    for r in range(nst):
        xs = x_ref[strip(r), :].astype(f32)
        ssum = xs if ssum is None else ssum + xs
    m = jnp.sum(ssum, axis=0, keepdims=True) * (1.0 / D)
    ssq = None
    for r in range(nst):
        xc = x_ref[strip(r), :].astype(f32) - m
        ssq = xc * xc if ssq is None else ssq + xc * xc
    var = jnp.sum(ssq, axis=0, keepdims=True) * (1.0 / D)
    rstd = lax.rsqrt(var + EPS)
    for r in range(nst):
        xnb_ref[strip(r), :] = ((x_ref[strip(r), :].astype(f32) - m) * rstd).astype(bf16)

    lane = lax.broadcasted_iota(jnp.int32, (ES, C), 1)
    fwd = fwd_ref[...]
    sgn = sgn_ref[...]

    i0 = step * SUB
    for sub in range(SUB):
        i = i0 + sub
        cols = slice(sub * C, (sub + 1) * C)
        h1 = jnp.dot(w1t_ref[...], xnb_ref[:, cols], preferred_element_type=f32)
        h1 = h1 * (0.5 + 0.5 * jnp.tanh(0.5 * h1))
        bout_ref[sub] = jnp.dot(w2t_ref[...], h1.astype(bf16), preferred_element_type=f32)

        for r in range(nst):
            rr = strip(r)
            sk = sk_ref[rr, :].astype(f32)
            kf = k_ref[rr, cols].astype(f32)
            ksh = kf * sk[:, 0:1]
            for t in range(1, 4):
                rolled = pltpu.roll(kf, t, 1)
                sh = jnp.where(lane < t, kprev_ref[t - 1, rr, :], rolled)
                kprev_ref[t - 1, rr, :] = rolled
                ksh = ksh + sh * sk[:, t:t + 1]
            kvb_ref[sub, rr, :] = (ksh * v_ref[rr, cols].astype(f32)).astype(bf16)

        u = jnp.dot(kvb_ref[sub], fwd, preferred_element_type=f32)
        hf_ref[i] = jnp.dot(h_ref[:, cols], fwd, preferred_element_type=f32)
        up = uprev_ref[...]
        uf_ref[i, :, :C] = up[:, :C] + sgn * u[:, C:]
        uf_ref[i, :, C:] = up[:, C:] - sgn * u[:, :C]
        uprev_ref[...] = u

    def ld(ref, idx, rows):
        return ref[idx, rows, :C], ref[idx, rows, C:]

    def cmul(a, b):
        return a[0] * b[0] - a[1] * b[1], a[0] * b[1] + a[1] * b[0]

    def cadd(a, b):
        return a[0] + b[0], a[1] + b[1]

    def st(idx, rows, val):
        yacc_ref[idx, rows, :C] = val[0]
        yacc_ref[idx, rows, C:] = val[1]

    for r in range(D // STRIP):
        rows = slice(r * STRIP, (r + 1) * STRIP)
        h0 = ld(hf_ref, 0, rows)
        st(0, rows, cmul(h0, ld(uf_ref, i0, rows)))
        st(1, rows, cadd(cmul(h0, ld(uf_ref, i0 + 1, rows)),
                         cmul(ld(hf_ref, i0 + 1, rows), ld(uf_ref, 0, rows))))

    def group(ka, nterms):
        for r in range(D // STRIP):
            rows = slice(r * STRIP, (r + 1) * STRIP)
            y0 = ld(yacc_ref, 0, rows)
            y1 = ld(yacc_ref, 1, rows)
            unext = ld(uf_ref, i0 + 1 - ka, rows)
            for n in range(nterms):
                hh = ld(hf_ref, ka + n, rows)
                ucur = ld(uf_ref, i0 - ka - n, rows)
                y1 = cadd(y1, cmul(hh, unext))
                y0 = cadd(y0, cmul(hh, ucur))
                unext = ucur
            st(0, rows, y0)
            st(1, rows, y1)

    def quad_body(j, carry):
        group(4 * j + 1, 4)
        return carry

    lax.fori_loop(0, step // 2, quad_body, 0)

    @pl.when(step % 2 == 1)
    def _():
        group(2 * step - 1, 2)

    for sub in range(SUB):
        cols = slice(sub * C, (sub + 1) * C)
        y = jnp.dot(yacc_ref[sub].astype(bf16), inv_ref[...], preferred_element_type=f32)
        ms = m[:, cols]
        rs = rstd[:, cols]
        for r in range(nst):
            rr = strip(r)
            xs = x_ref[rr, cols].astype(f32)
            xn = (xs - ms) * rs
            yy = y[rr, :] + kvb_ref[sub, rr, :].astype(f32) * d_ref[rr, :].astype(f32)
            o_ref[rr, cols] = (xs + xn * yy + bout_ref[sub, rr, :]).astype(o_ref.dtype)


@jax.jit
def pallas_parallel_sum__ssm_conv_h3__dense_activation_silu__prompt_kernel(
    A_q: jax.Array,
    A_k: jax.Array,
    A_v: jax.Array,
    A_shift_k: jax.Array,
    A_ssm_k: jax.Array,
    A_ssm_D: jax.Array,
    B_x: jax.Array,
    B_w1: jax.Array,
    B_w2: jax.Array,
):
    B, S, D = A_q.shape
    assert B == 1 and S % W == 0 and SUB == 2
    F = B_w1.shape[1]
    nb = S // C
    bf16 = jnp.bfloat16

    xt = A_q.reshape(S, D).T
    kt = A_k.reshape(S, D).T
    vt = A_v.reshape(S, D).T
    d2 = A_ssm_D.reshape(D, 1)
    w2t = B_w2.T

    fwd, inv, sgn = _dft_constants()
    fwd = jnp.asarray(fwd, dtype=bf16)
    inv = jnp.asarray(inv, dtype=bf16)
    sgn = jnp.asarray(sgn, dtype=jnp.float32)

    col = lambda i: (0, i)
    const = lambda i: (0, 0)
    out = pl.pallas_call(
        _kernel,
        grid=(S // W,),
        in_specs=[
            pl.BlockSpec((D, W), col),
            pl.BlockSpec((D, W), col),
            pl.BlockSpec((D, W), col),
            pl.BlockSpec((D, 4), const),
            pl.BlockSpec((D, W), col),
            pl.BlockSpec((D, 1), const),
            pl.BlockSpec((D, F), const),
            pl.BlockSpec((D, F), const),
            pl.BlockSpec((C, N2), const),
            pl.BlockSpec((N2, C), const),
            pl.BlockSpec((1, C), const),
        ],
        out_specs=pl.BlockSpec((D, W), col),
        out_shape=jax.ShapeDtypeStruct((D, S), A_q.dtype),
        scratch_shapes=[
            pltpu.VMEM((nb, D, N2), jnp.float32),
            pltpu.VMEM((nb, D, N2), jnp.float32),
            pltpu.VMEM((D, N2), jnp.float32),
            pltpu.VMEM((3, D, C), jnp.float32),
            pltpu.VMEM((SUB, D, N2), jnp.float32),
            pltpu.VMEM((F, D), bf16),
            pltpu.VMEM((D, W), bf16),
            pltpu.VMEM((SUB, D, C), bf16),
            pltpu.VMEM((SUB, D, C), jnp.float32),
        ],
        compiler_params=pltpu.CompilerParams(
            dimension_semantics=("arbitrary",),
            vmem_limit_bytes=100 * 1024 * 1024,
        ),
    )(xt, kt, vt, A_shift_k, A_ssm_k, d2, B_w1, w2t, fwd, inv, sgn)
    return out.T.reshape(B, S, D)
```
